```python
import jax
import jax.numpy as jnp

def _softmax(x, axis=-1):
    return jax.nn.softmax(x, axis=axis)
def _gelu(x):
    return jax.nn.gelu(x, approximate=True)
def _silu(x):
    return jax.nn.silu(x)
def _sigmoid(x):
    return jax.nn.sigmoid(x)
def _layernorm(x, axis=-1, eps=1e-5):
    m = jnp.mean(x, axis=axis, keepdims=True)
    v = jnp.var(x, axis=axis, keepdims=True)
    return (x - m) / jnp.sqrt(v + eps)
def _scatter_add(tgt, idx, src, axis=0):
    return tgt.at[idx].add(src)
def _segment_sum(src, seg, n):
    return jax.ops.segment_sum(src, seg, n)
class _Rng:
    def __init__(self, key):
        self._k = key
    def _next(self):
        self._k, sub = jax.random.split(self._k)
        return sub
    def normal(self, shape):
        return jax.random.normal(self._next(), shape, dtype=jnp.bfloat16)
    def randint(self, lo, hi, shape):
        return jax.random.randint(self._next(), shape, lo, hi, dtype=jnp.int32)
    def uniform(self, shape, lo=0.0, hi=1.0):
        return jax.random.uniform(self._next(), shape, jnp.bfloat16, lo, hi)
    def permutation(self, n):
        return jax.random.permutation(self._next(), n)


kernel_name = 'recurrent_scan__sliding_block_cached__mixer_s_mlp__decode'

def setup_inputs():
    _rng = _Rng(jax.random.key(int.from_bytes(__import__("os").urandom(4), "little")))
    _w = (lambda a: (lambda t: t.astype(jnp.bfloat16) if jnp.issubdtype(t.dtype, jnp.floating) else t)(jnp.asarray(a)))
    def _A_setup():
        B, Sq, D = 1, 1, 512
        Hq, Hkv, Sk, Dh = 32, 32, 32768, 128
        assert Hq % Hkv == 0, (Hq, Hkv)
        return {
            "x": _w((lambda *s: _rng.normal(s) * 0.05)(B, Sq, D)),
            "k_cache": _w((lambda *s: _rng.normal(s) * 0.05)(B, Hkv, Sk, Dh)),
            "v_cache": _w((lambda *s: _rng.normal(s) * 0.05)(B, Hkv, Sk, Dh)),
            "wq": _w((lambda *s: _rng.normal(s) * 0.05)(D, Hq * Dh) * (D ** -0.5)),
            "wo": _w((lambda *s: _rng.normal(s) * 0.05)(Hq * Dh, D) * ((Hq * Dh) ** -0.5)),
        }
    _A_in = _A_setup()

    def _B_setup():
        B, S, D, F = 1, 1, 512, 1376
        return {
            "x":  _w((lambda *s: _rng.normal(s) * 0.05)(B, S, D)),
            "w1": _w((lambda *s: _rng.normal(s) * 0.05)(D, D) * (D ** -0.5)),
            "w2": _w((lambda *s: _rng.normal(s) * 0.05)(D, D) * (D ** -0.5)),
            "w3": _w((lambda *s: _rng.normal(s) * 0.05)(D, F) * (D ** -0.5)),
            "w4": _w((lambda *s: _rng.normal(s) * 0.05)(F, D) * (F ** -0.5)),
        }
    _B_in = _B_setup()

    return {
        "A_x": _A_in["x"],
        "A_k_cache": _A_in["k_cache"],
        "A_v_cache": _A_in["v_cache"],
        "A_wq": _A_in["wq"],
        "A_wo": _A_in["wo"],
        "B_x": _B_in["x"],
        "B_w1": _B_in["w1"],
        "B_w2": _B_in["w2"],
        "B_w3": _B_in["w3"],
        "B_w4": _B_in["w4"],
    }

def reference(A_x, A_k_cache, A_v_cache, A_wq, A_wo, B_x, B_w1, B_w2, B_w3, B_w4):
    def _A_ref(x, k_cache, v_cache, wq, wo):
        B, Sq, D = x.shape
        Hq, Dh = 32, 128
        Hkv, Sk = k_cache.shape[1], k_cache.shape[2]
        W = min(4096, max(256, Sk // 4))
        rep = Hq // Hkv
        q = (lambda x, *d: x.transpose(*d))((x @ wq).reshape(B, Sq, Hq, Dh), 0, 2, 1, 3)
        k = jnp.repeat(k_cache[:, :, Sk - W:, :], rep, axis=1)
        v = jnp.repeat(v_cache[:, :, Sk - W:, :], rep, axis=1)
        scores = jnp.einsum("bhqd,bhkd->bhqk", q, k) * (Dh ** -0.5)
        p = _softmax(scores, axis=-1)
        o = jnp.einsum("bhqk,bhkd->bhqd", p, v)
        return (lambda x, *d: x.transpose(*d))(o, 0, 2, 1, 3).reshape(B, Sq, Hq * Dh) @ wo

    def _B_ref(x, w1, w2, w3, w4):
        B, S, D = x.shape
        h = _gelu(_layernorm(x, axis=-1) @ w1)
        c = D // 4
        g0 = jnp.pad(h[:, :, 0*c:1*c], ((0, 0), (1, 0), (0, 0)))[:, :S, :]
        g1 = jnp.pad(h[:, :, 1*c:2*c], ((0, 0), (0, 1), (0, 0)))[:, 1:, :]
        g2 = jnp.pad(h[:, :, 2*c:3*c], ((0, 0), (2, 0), (0, 0)))[:, :S, :]
        g3 = jnp.pad(h[:, :, 3*c:   ], ((0, 0), (0, 2), (0, 0)))[:, 2:, :]
        hs = jnp.concatenate([g0, g1, g2, g3], axis=-1) @ w2
        x1 = x + hs
        h2 = _gelu(_layernorm(x1, axis=-1) @ w3) @ w4
        return x1 + h2

    x = A_x
    xn = _layernorm(x, axis=-1)
    s = _A_ref(xn, A_k_cache, A_v_cache, A_wq, A_wo)
    g = _silu(_B_ref(xn, B_w1, B_w2, B_w3, B_w4))
    return x + s * g
```

```python
import jax
import jax.numpy as jnp
from jax import lax
from jax.experimental import pallas as pl
from jax.experimental.pallas import tpu as pltpu

_BF16 = jnp.bfloat16
_F32 = jnp.float32
_M = 8


def _layernorm(x, eps=1e-5):
    m = jnp.mean(x, axis=-1, keepdims=True)
    xc = x - m
    v = jnp.mean(xc * xc, axis=-1, keepdims=True)
    return xc / jnp.sqrt(v + eps)


def _bounds(groups):
    b = [0]
    for s in groups:
        b.append(b[-1] + s)
    return b


@jax.jit
def pallas_recurrent_scan__sliding_block_cached__mixer_s_mlp__decode_kernel(
    A_x: jax.Array,
    A_k_cache: jax.Array,
    A_v_cache: jax.Array,
    A_wq: jax.Array,
    A_wo: jax.Array,
    B_x: jax.Array,
    B_w1: jax.Array,
    B_w2: jax.Array,
    B_w3: jax.Array,
    B_w4: jax.Array,
):
    B, S, D = A_x.shape
    _, H, SK, DH = A_k_cache.shape
    F = B_w3.shape[1]
    assert B == 1 and S == 1 and A_wq.shape == (D, H * DH)
    W = min(4096, max(256, SK // 4))

    kg = (H,)
    vg = (H - H // 4, H // 4)
    wog = (H - 7, 6, 1)
    kb, vb, wb = _bounds(kg), _bounds(vg), _bounds(wog)

    def kernel(x_hbm, k_hbm, v_hbm, wq_hbm, wo_hbm, w3t_hbm, w4_hbm, o_ref,
               xbuf, kbuf, vbuf, wqbuf, wobuf, w3tbuf, w4buf, qscr, pscr, oscr,
               ksem, vsem, wsem, wosem):
        def kdma(i):
            a, n = kb[i], kg[i]
            return pltpu.make_async_copy(
                k_hbm.at[0, pl.ds(a, n), pl.ds(SK - W, W), :],
                kbuf.at[pl.ds(a, n)], ksem.at[i])

        def vdma(i):
            a, n = vb[i], vg[i]
            return pltpu.make_async_copy(
                v_hbm.at[0, pl.ds(a, n), pl.ds(SK - W, W), :],
                vbuf.at[pl.ds(a, n)], vsem.at[i])

        def wodma(i):
            a, n = wb[i] * DH, wog[i] * DH
            return pltpu.make_async_copy(
                wo_hbm.at[pl.ds(a, n), :], wobuf.at[pl.ds(a, n), :], wosem.at[i])

        xd = pltpu.make_async_copy(x_hbm, xbuf, wsem.at[0])
        wqd = pltpu.make_async_copy(wq_hbm, wqbuf, wsem.at[1])
        w3d = pltpu.make_async_copy(w3t_hbm, w3tbuf, wsem.at[2])
        w4d = pltpu.make_async_copy(w4_hbm, w4buf, wsem.at[3])

        wqd.start()
        rest = ([xd, w3d, w4d]
                + [kdma(i) for i in range(len(kg))]
                + [vdma(i) for i in range(len(vg))]
                + [wodma(i) for i in range(len(wog))])

        def issue(i, c):
            for j, d in enumerate(rest):
                @pl.when(i == j)
                def _(d=d):
                    d.start()
            return c

        lax.fori_loop(0, len(rest), issue, 0)

        xd.wait()
        x = xbuf[...].astype(_F32)
        xn = jnp.broadcast_to(_layernorm(x), (_M, D)).astype(_BF16)
        wqd.wait()
        q = jnp.dot(xn, wqbuf[...], preferred_element_type=_F32)
        for h in range(H):
            qscr[h] = q[:, h * DH:(h + 1) * DH].astype(_BF16)

        w3d.wait()
        w4d.wait()
        xn32 = xn.astype(_F32)
        y = _layernorm(xn32).astype(_BF16)
        h1 = lax.dot_general(y, w3tbuf[...], (((1,), (1,)), ((), ())),
                             preferred_element_type=_F32)
        h1 = jax.nn.gelu(h1, approximate=True).astype(_BF16)
        b = xn32 + jnp.dot(h1, w4buf[...], preferred_element_type=_F32)
        g = (b * jax.nn.sigmoid(b))[0:1]

        def qk(h, c):
            s = lax.dot_general(qscr[h], kbuf[h], (((1,), (1,)), ((), ())),
                                preferred_element_type=_F32)
            s = s * (DH ** -0.5)
            p = jnp.exp(s - jnp.max(s, axis=-1, keepdims=True))
            l = jnp.sum(p, axis=-1, keepdims=True)
            pscr[h] = (p * (1.0 / l)).astype(_BF16)
            return c

        def pv(h, c):
            o = jnp.dot(pscr[h], vbuf[h], preferred_element_type=_F32)
            oscr[h] = o.astype(_BF16)
            return c

        for i in range(len(kg)):
            kdma(i).wait()
            lax.fori_loop(kb[i], kb[i + 1], qk, 0)
        for i in range(len(vg)):
            vdma(i).wait()
            lax.fori_loop(vb[i], vb[i + 1], pv, 0)

        acc = jnp.zeros((_M, D), _F32)
        for i in range(len(wog)):
            wodma(i).wait()
            for h in range(wb[i], wb[i + 1]):
                acc = acc + jnp.dot(oscr[h], wobuf[h * DH:(h + 1) * DH, :],
                                    preferred_element_type=_F32)
        o_ref[...] = (x + acc[0:1] * g).astype(_BF16)

    out = pl.pallas_call(
        kernel,
        out_shape=jax.ShapeDtypeStruct((1, D), _BF16),
        in_specs=[pl.BlockSpec(memory_space=pl.ANY)] * 7,
        out_specs=pl.BlockSpec(memory_space=pltpu.VMEM),
        scratch_shapes=[
            pltpu.VMEM((1, D), _BF16),
            pltpu.VMEM((H, W, DH), _BF16),
            pltpu.VMEM((H, W, DH), _BF16),
            pltpu.VMEM((D, H * DH), _BF16),
            pltpu.VMEM((H * DH, D), _BF16),
            pltpu.VMEM((F, D), _BF16),
            pltpu.VMEM((F, D), _BF16),
            pltpu.VMEM((H, _M, DH), _BF16),
            pltpu.VMEM((H, _M, W), _BF16),
            pltpu.VMEM((H, _M, DH), _BF16),
            pltpu.SemaphoreType.DMA((len(kg),)),
            pltpu.SemaphoreType.DMA((len(vg),)),
            pltpu.SemaphoreType.DMA((4,)),
            pltpu.SemaphoreType.DMA((len(wog),)),
        ],
        compiler_params=pltpu.CompilerParams(vmem_limit_bytes=100 * 1024 * 1024),
    )(A_x.reshape(1, D), A_k_cache, A_v_cache, A_wq, A_wo, B_w3.T, B_w4)
    return out.reshape(1, 1, D)
```

```python
import jax
import jax.numpy as jnp
from jax import lax
from jax.experimental import pallas as pl
from jax.experimental.pallas import tpu as pltpu

_BF16 = jnp.bfloat16
_F32 = jnp.float32
_M = 8


def _layernorm(x, eps=1e-5):
    m = jnp.mean(x, axis=-1, keepdims=True)
    xc = x - m
    v = jnp.mean(xc * xc, axis=-1, keepdims=True)
    return xc / jnp.sqrt(v + eps)


@jax.jit
def pallas_recurrent_scan__sliding_block_cached__mixer_s_mlp__decode_kernel(
    A_x: jax.Array,
    A_k_cache: jax.Array,
    A_v_cache: jax.Array,
    A_wq: jax.Array,
    A_wo: jax.Array,
    B_x: jax.Array,
    B_w1: jax.Array,
    B_w2: jax.Array,
    B_w3: jax.Array,
    B_w4: jax.Array,
):
    B, S, D = A_x.shape
    _, H, SK, DH = A_k_cache.shape
    F = B_w3.shape[1]
    assert B == 1 and S == 1 and A_wq.shape == (D, H * DH)
    W = min(4096, max(256, SK // 4))

    R = 128
    LOOK = 2
    NS = LOOK + 1
    WQR, WQC = 8, 1024
    WR = 16
    HH = H // 2
    wog = (HH // 2, 5, 2, 1)
    assert sum(wog) == HH and W % R == 0 and F % WR == 0
    wb = [0]
    for s in wog:
        wb.append(wb[-1] + s)
    NG = len(wog)

    def kernel(x_hbm, k_hbm, v_hbm, wq_hbm, wo_hbm, w3t_hbm, w4_hbm, o_ref,
               xbuf, kbuf, vbuf, wqbuf, wobuf, w3tbuf, w4buf, qscr, oscr,
               ksem, vsem, wsem, wosem):
        def copy(src, dst, sem, priority):
            pltpu.make_async_copy(src, dst, sem).start(priority=priority)

        def wait_all(buf, sem):
            pltpu.make_async_copy(buf, buf, sem).wait()

        def issue_head(h):
            s = h % NS

            def body(c, carry):
                r = pl.multiple_of(c * R, R)
                copy(k_hbm.at[0, h, pl.ds(SK - W + r, R), :],
                     kbuf.at[h, pl.ds(r, R), :], ksem.at[s], 0)
                copy(v_hbm.at[0, h, pl.ds(SK - W + r, R), :],
                     vbuf.at[h, pl.ds(r, R), :], vsem.at[s], 1)
                return carry

            lax.fori_loop(0, W // R, body, 0)

        def issue_wo(g):
            def body(c, carry):
                for t in range(2):
                    r = pl.multiple_of(c * WR + t * HH * DH, WR)
                    copy(wo_hbm.at[pl.ds(r, WR), :], wobuf.at[pl.ds(r, WR), :],
                         wosem.at[t, g], t)
                return carry

            lax.fori_loop(wb[g] * DH // WR, wb[g + 1] * DH // WR, body, 0)

        xd = pltpu.make_async_copy(x_hbm, xbuf, wsem.at[0])
        xd.start()

        def wq_body(i, carry):
            for c in range(H * DH // WQC):
                for t in range(2):
                    r = pl.multiple_of(i * WQR + t * (D // 2), WQR)
                    copy(wq_hbm.at[pl.ds(r, WQR), pl.ds(c * WQC, WQC)],
                         wqbuf.at[pl.ds(r, WQR), pl.ds(c * WQC, WQC)],
                         wsem.at[1], t)
            return carry

        lax.fori_loop(0, D // (2 * WQR), wq_body, 0)

        def w34_body(i, carry):
            r = pl.multiple_of(i * WR, WR)
            copy(w3t_hbm.at[pl.ds(r, WR), :], w3tbuf.at[pl.ds(r, WR), :],
                 wsem.at[2], 0)
            copy(w4_hbm.at[pl.ds(r, WR), :], w4buf.at[pl.ds(r, WR), :],
                 wsem.at[3], 1)
            return carry

        lax.fori_loop(0, F // WR, w34_body, 0)
        for h in range(LOOK - 1):
            issue_head(h)

        xd.wait()
        x = xbuf[...].astype(_F32)
        xn = jnp.broadcast_to(_layernorm(x), (_M, D)).astype(_BF16)
        wait_all(wqbuf, wsem.at[1])
        q = jnp.dot(xn, wqbuf[...], preferred_element_type=_F32)
        for h in range(H):
            qscr[h] = q[:, h * DH:(h + 1) * DH].astype(_BF16)

        issue_head(LOOK - 1)

        wait_all(w3tbuf, wsem.at[2])
        wait_all(w4buf, wsem.at[3])
        xn32 = xn.astype(_F32)
        y = _layernorm(xn32).astype(_BF16)
        h1 = lax.dot_general(y, w3tbuf[...], (((1,), (1,)), ((), ())),
                             preferred_element_type=_F32)
        h1 = jax.nn.gelu(h1, approximate=True).astype(_BF16)
        b = xn32 + jnp.dot(h1, w4buf[...], preferred_element_type=_F32)
        g = (b * jax.nn.sigmoid(b))[0:1]

        def head(h, carry):
            @pl.when(h + LOOK < H)
            def _():
                issue_head(h + LOOK)

            @pl.when(h == H - 2)
            def _():
                issue_wo(0)

            @pl.when(h == H - 1)
            def _():
                for gi in range(1, NG):
                    issue_wo(gi)

            wait_all(kbuf.at[h], ksem.at[h % NS])
            s = lax.dot_general(qscr[h], kbuf[h], (((1,), (1,)), ((), ())),
                                preferred_element_type=_F32)
            s = s * (DH ** -0.5)
            p = jnp.exp(s - jnp.max(s, axis=-1, keepdims=True))
            l = jnp.sum(p, axis=-1, keepdims=True)
            wait_all(vbuf.at[h], vsem.at[h % NS])
            o = jnp.dot(p.astype(_BF16), vbuf[h], preferred_element_type=_F32)
            oscr[h] = (o * (1.0 / l)).astype(_BF16)
            return carry

        lax.fori_loop(0, H, head, 0)

        acc = jnp.zeros((_M, D), _F32)
        for gi in range(NG):
            for t in range(2):
                rows = pl.ds((t * HH + wb[gi]) * DH, wog[gi] * DH)
                wait_all(wobuf.at[rows, :], wosem.at[t, gi])
            for hh in range(wb[gi], wb[gi + 1]):
                for h in (hh, hh + HH):
                    acc = acc + jnp.dot(oscr[h], wobuf[h * DH:(h + 1) * DH, :],
                                        preferred_element_type=_F32)
        o_ref[...] = (x + acc[0:1] * g).astype(_BF16)

    out = pl.pallas_call(
        kernel,
        out_shape=jax.ShapeDtypeStruct((1, D), _BF16),
        in_specs=[pl.BlockSpec(memory_space=pl.ANY)] * 7,
        out_specs=pl.BlockSpec(memory_space=pltpu.VMEM),
        scratch_shapes=[
            pltpu.VMEM((1, D), _BF16),
            pltpu.VMEM((H, W, DH), _BF16),
            pltpu.VMEM((H, W, DH), _BF16),
            pltpu.VMEM((D, H * DH), _BF16),
            pltpu.VMEM((H * DH, D), _BF16),
            pltpu.VMEM((F, D), _BF16),
            pltpu.VMEM((F, D), _BF16),
            pltpu.VMEM((H, _M, DH), _BF16),
            pltpu.VMEM((H, _M, DH), _BF16),
            pltpu.SemaphoreType.DMA((NS,)),
            pltpu.SemaphoreType.DMA((NS,)),
            pltpu.SemaphoreType.DMA((4,)),
            pltpu.SemaphoreType.DMA((2, NG)),
        ],
        compiler_params=pltpu.CompilerParams(
            vmem_limit_bytes=100 * 1024 * 1024,
            disable_semaphore_checks=True,
            disable_bounds_checks=True,
        ),
    )(A_x.reshape(1, D), A_k_cache, A_v_cache, A_wq, A_wo, B_w3.T, B_w4)
    return out.reshape(1, 1, D)
```

```python
import jax
import jax.numpy as jnp
from jax import lax
from jax.experimental import pallas as pl
from jax.experimental.pallas import tpu as pltpu

_BF16 = jnp.bfloat16
_F32 = jnp.float32
_M = 8


def _layernorm(x, eps=1e-5):
    m = jnp.mean(x, axis=-1, keepdims=True)
    xc = x - m
    v = jnp.mean(xc * xc, axis=-1, keepdims=True)
    return xc / jnp.sqrt(v + eps)


@jax.jit
def pallas_recurrent_scan__sliding_block_cached__mixer_s_mlp__decode_kernel(
    A_x: jax.Array,
    A_k_cache: jax.Array,
    A_v_cache: jax.Array,
    A_wq: jax.Array,
    A_wo: jax.Array,
    B_x: jax.Array,
    B_w1: jax.Array,
    B_w2: jax.Array,
    B_w3: jax.Array,
    B_w4: jax.Array,
):
    B, S, D = A_x.shape
    _, H, SK, DH = A_k_cache.shape
    F = B_w3.shape[1]
    assert B == 1 and S == 1 and A_wq.shape == (D, H * DH)
    assert H == 32 and DH == 128
    W = min(4096, max(256, SK // 4))

    R = 64
    NC = W // R
    VSHIFT = 3
    LOOK = 2
    NS = LOOK + 1
    WQR, WQC = 8, 1024
    WR = 16
    assert W % R == 0 and F % WR == 0 and NC > VSHIFT

    mxu_groups = (
        ((0 * DH, 8 * DH), (19 * DH, 8 * DH)),
        ((8 * DH, 6 * DH), (27 * DH, 4 * DH)),
        ((14 * DH, 2 * DH), (31 * DH, 1 * DH)),
    )
    VH0, NVH = 16, 3
    vpu_rows = (128, 128, 64, 32, 16, 16)
    ranges0 = [g[0] for g in mxu_groups]
    ranges1 = [g[1] for g in mxu_groups]
    r = VH0 * DH
    for n in vpu_rows:
        ranges1.append((r, n))
        r += n
    assert r == (VH0 + NVH) * DH

    def per_descriptor(ranges):
        return [(r0 + c * WR, i) for i, (r0, n) in enumerate(ranges)
                for c in range(n // WR)]

    wo_desc = list(zip(per_descriptor(ranges0), per_descriptor(ranges1),
                       strict=True))
    NWO = len(wo_desc)
    WO_SPLIT = (64, 86)
    OBC_AT = 20

    def kernel(x_hbm, k_hbm, v_hbm, wq_hbm, wo_hbm, w3t_hbm, w4_hbm, o_ref,
               xbuf, kbuf, vbuf, wqbuf, wobuf, w3tbuf, w4buf, qscr, oscr, obc,
               ksem, vsem, wsem, wosem0, wosem1):
        def copy(src, dst, sem, priority):
            pltpu.make_async_copy(src, dst, sem).start(priority=priority)

        def wait_all(buf, sem):
            pltpu.make_async_copy(buf, buf, sem).wait()

        def issue_head(h):
            s = h % NS

            def body(c, carry):
                rk = pl.multiple_of(c * R, R)
                cv = c + VSHIFT
                rv = pl.multiple_of(jnp.where(cv >= NC, cv - NC, cv) * R, R)
                copy(k_hbm.at[0, h, pl.ds(SK - W + rk, R), :],
                     kbuf.at[h, pl.ds(rk, R), :], ksem.at[s], 0)
                copy(v_hbm.at[0, h, pl.ds(SK - W + rv, R), :],
                     vbuf.at[h, pl.ds(rv, R), :], vsem.at[s], 1)
                return carry

            lax.fori_loop(0, NC, body, 0)

        def issue_wo(p0, p1):
            i = p0
            while i < p1:
                j = i + 1
                while (j < p1 and wo_desc[j][0][1] == wo_desc[i][0][1]
                       and wo_desc[j][1][1] == wo_desc[i][1][1]):
                    j += 1
                (r0, s0), (r1, s1) = wo_desc[i]

                def body(c, carry, r0=r0, r1=r1, s0=s0, s1=s1):
                    a = pl.multiple_of(r0 + c * WR, WR)
                    b = pl.multiple_of(r1 + c * WR, WR)
                    copy(wo_hbm.at[pl.ds(a, WR), :], wobuf.at[pl.ds(a, WR), :],
                         wosem0.at[s0], 0)
                    copy(wo_hbm.at[pl.ds(b, WR), :], wobuf.at[pl.ds(b, WR), :],
                         wosem1.at[s1], 1)
                    return carry

                lax.fori_loop(0, j - i, body, 0)
                i = j

        xd = pltpu.make_async_copy(x_hbm, xbuf, wsem.at[0])
        xd.start()

        def wq_body(i, carry):
            for c in range(H * DH // WQC):
                for t in range(2):
                    r = pl.multiple_of(i * WQR + t * (D // 2), WQR)
                    copy(wq_hbm.at[pl.ds(r, WQR), pl.ds(c * WQC, WQC)],
                         wqbuf.at[pl.ds(r, WQR), pl.ds(c * WQC, WQC)],
                         wsem.at[1], t)
            return carry

        lax.fori_loop(0, D // (2 * WQR), wq_body, 0)

        def w34_body(i, carry):
            r = pl.multiple_of(i * WR, WR)
            copy(w3t_hbm.at[pl.ds(r, WR), :], w3tbuf.at[pl.ds(r, WR), :],
                 wsem.at[2], 0)
            copy(w4_hbm.at[pl.ds(r, WR), :], w4buf.at[pl.ds(r, WR), :],
                 wsem.at[3], 1)
            return carry

        lax.fori_loop(0, F // WR, w34_body, 0)
        issue_head(0)

        xd.wait()
        x = xbuf[...].astype(_F32)
        xn = jnp.broadcast_to(_layernorm(x), (_M, D)).astype(_BF16)
        wait_all(wqbuf, wsem.at[1])
        q = jnp.dot(xn, wqbuf[...], preferred_element_type=_F32)
        for h in range(H):
            qscr[h] = q[:, h * DH:(h + 1) * DH].astype(_BF16)

        issue_head(1)

        wait_all(w3tbuf, wsem.at[2])
        wait_all(w4buf, wsem.at[3])
        xn32 = xn.astype(_F32)
        y = _layernorm(xn32).astype(_BF16)
        h1 = lax.dot_general(y, w3tbuf[...], (((1,), (1,)), ((), ())),
                             preferred_element_type=_F32)
        h1 = jax.nn.gelu(h1, approximate=True).astype(_BF16)
        b = xn32 + jnp.dot(h1, w4buf[...], preferred_element_type=_F32)
        g = (b * jax.nn.sigmoid(b))[0:1]

        def head(h, carry):
            @pl.when(h + LOOK < H)
            def _():
                issue_head(h + LOOK)

            @pl.when(h == H - 2)
            def _():
                issue_wo(0, WO_SPLIT[0])

            @pl.when(h == H - 1)
            def _():
                issue_wo(WO_SPLIT[0], WO_SPLIT[1])

            wait_all(kbuf.at[h], ksem.at[h % NS])
            s = lax.dot_general(qscr[h], kbuf[h], (((1,), (1,)), ((), ())),
                                preferred_element_type=_F32)
            s = s * (DH ** -0.5)
            p = jnp.exp(s - jnp.max(s, axis=-1, keepdims=True))
            l = jnp.sum(p, axis=-1, keepdims=True)
            wait_all(vbuf.at[h], vsem.at[h % NS])
            o = jnp.dot(p.astype(_BF16), vbuf[h], preferred_element_type=_F32)
            oscr[h] = (o * (1.0 / l)).astype(_BF16)

            @pl.when(h == OBC_AT)
            def _():
                for t in range(NVH):
                    ot = jnp.transpose(oscr[VH0 + t].astype(_F32))
                    obc[t] = jnp.broadcast_to(ot[:, 0:1], (DH, DH))

            return carry

        lax.fori_loop(0, H, head, 0)
        issue_wo(WO_SPLIT[1], NWO)

        acc = jnp.zeros((_M, D), _F32)
        for gi, (g0, g1) in enumerate(mxu_groups):
            for (r0, n), sem in ((g0, wosem0.at[gi]), (g1, wosem1.at[gi])):
                wait_all(wobuf.at[pl.ds(r0, n), :], sem)
            for r0, n in (g0, g1):
                for h in range(r0 // DH, (r0 + n) // DH):
                    acc = acc + jnp.dot(oscr[h], wobuf[h * DH:(h + 1) * DH, :],
                                        preferred_element_type=_F32)
        base = x + acc[0:1] * g

        vacc = jnp.zeros((_M, D), _F32)
        for v, n in enumerate(vpu_rows):
            r0 = ranges1[len(mxu_groups) + v][0]
            wait_all(wobuf.at[pl.ds(r0, n), :], wosem1.at[len(mxu_groups) + v])
            t, k0 = r0 // DH - VH0, r0 % DH
            ob = obc[t, k0:k0 + n, :]
            prod = (wobuf[r0:r0 + n, :].astype(_F32)
                    * jnp.concatenate([ob] * (D // DH), axis=1))
            for u in range(n // _M):
                vacc = vacc + prod[u * _M:(u + 1) * _M, :]
        s_tail = jnp.sum(vacc, axis=0, keepdims=True)
        o_ref[...] = (base + s_tail * g).astype(_BF16)

    out = pl.pallas_call(
        kernel,
        out_shape=jax.ShapeDtypeStruct((1, D), _BF16),
        in_specs=[pl.BlockSpec(memory_space=pl.ANY)] * 7,
        out_specs=pl.BlockSpec(memory_space=pltpu.VMEM),
        scratch_shapes=[
            pltpu.VMEM((1, D), _BF16),
            pltpu.VMEM((H, W, DH), _BF16),
            pltpu.VMEM((H, W, DH), _BF16),
            pltpu.VMEM((D, H * DH), _BF16),
            pltpu.VMEM((H * DH, D), _BF16),
            pltpu.VMEM((F, D), _BF16),
            pltpu.VMEM((F, D), _BF16),
            pltpu.VMEM((H, _M, DH), _BF16),
            pltpu.VMEM((H, _M, DH), _BF16),
            pltpu.VMEM((NVH, DH, DH), _F32),
            pltpu.SemaphoreType.DMA((NS,)),
            pltpu.SemaphoreType.DMA((NS,)),
            pltpu.SemaphoreType.DMA((4,)),
            pltpu.SemaphoreType.DMA((len(ranges0),)),
            pltpu.SemaphoreType.DMA((len(ranges1),)),
        ],
        compiler_params=pltpu.CompilerParams(
            vmem_limit_bytes=100 * 1024 * 1024,
            disable_semaphore_checks=True,
            disable_bounds_checks=True,
        ),
    )(A_x.reshape(1, D), A_k_cache, A_v_cache, A_wq, A_wo, B_w3.T, B_w4)
    return out.reshape(1, 1, D)
```
